```python
import jax
import jax.numpy as jnp

def _softmax(x, axis=-1):
    return jax.nn.softmax(x, axis=axis)
def _gelu(x):
    return jax.nn.gelu(x, approximate=True)
def _silu(x):
    return jax.nn.silu(x)
def _sigmoid(x):
    return jax.nn.sigmoid(x)
def _layernorm(x, axis=-1, eps=1e-5):
    m = jnp.mean(x, axis=axis, keepdims=True)
    v = jnp.var(x, axis=axis, keepdims=True)
    return (x - m) / jnp.sqrt(v + eps)
def _scatter_add(tgt, idx, src, axis=0):
    return tgt.at[idx].add(src)
def _segment_sum(src, seg, n):
    return jax.ops.segment_sum(src, seg, n)
class _Rng:
    def __init__(self, key):
        self._k = key
    def _next(self):
        self._k, sub = jax.random.split(self._k)
        return sub
    def normal(self, shape):
        return jax.random.normal(self._next(), shape, dtype=jnp.bfloat16)
    def randint(self, lo, hi, shape):
        return jax.random.randint(self._next(), shape, lo, hi, dtype=jnp.int32)
    def uniform(self, shape, lo=0.0, hi=1.0):
        return jax.random.uniform(self._next(), shape, jnp.bfloat16, lo, hi)
    def permutation(self, n):
        return jax.random.permutation(self._next(), n)


kernel_name = 'concat_heads__sliding_block_cached__sliding_block_cached__decode'

def _fwd_setup_inputs():
    _rng = _Rng(jax.random.key(int.from_bytes(__import__("os").urandom(4), "little")))
    _w = (lambda a: (lambda t: t.astype(jnp.bfloat16) if jnp.issubdtype(t.dtype, jnp.floating) else t)(jnp.asarray(a)))
    def _A_setup():
        B, Sq, D = 2, 1, 448
        Hq, Hkv, Sk, Dh = 16, 8, 4096, 256
        assert Hq % Hkv == 0, (Hq, Hkv)
        return {
            "x": _w((lambda *s: _rng.normal(s) * 0.05)(B, Sq, D)),
            "k_cache": _w((lambda *s: _rng.normal(s) * 0.05)(B, Hkv, Sk, Dh)),
            "v_cache": _w((lambda *s: _rng.normal(s) * 0.05)(B, Hkv, Sk, Dh)),
            "wq": _w((lambda *s: _rng.normal(s) * 0.05)(D, Hq * Dh) * (D ** -0.5)),
            "wo": _w((lambda *s: _rng.normal(s) * 0.05)(Hq * Dh, D) * ((Hq * Dh) ** -0.5)),
        }
    _A_in = _A_setup()

    def _B_setup():
        B, Sq, D = 2, 1, 448
        Hq, Hkv, Sk, Dh = 16, 8, 4096, 256
        assert Hq % Hkv == 0, (Hq, Hkv)
        return {
            "x": _w((lambda *s: _rng.normal(s) * 0.05)(B, Sq, D)),
            "k_cache": _w((lambda *s: _rng.normal(s) * 0.05)(B, Hkv, Sk, Dh)),
            "v_cache": _w((lambda *s: _rng.normal(s) * 0.05)(B, Hkv, Sk, Dh)),
            "wq": _w((lambda *s: _rng.normal(s) * 0.05)(D, Hq * Dh) * (D ** -0.5)),
            "wo": _w((lambda *s: _rng.normal(s) * 0.05)(Hq * Dh, D) * ((Hq * Dh) ** -0.5)),
        }
    _B_in = _B_setup()

    return {
        "A_x": _A_in["x"],
        "A_k_cache": _A_in["k_cache"],
        "A_v_cache": _A_in["v_cache"],
        "A_wq": _A_in["wq"],
        "A_wo": _A_in["wo"],
        "B_x": _B_in["x"],
        "B_k_cache": _B_in["k_cache"],
        "B_v_cache": _B_in["v_cache"],
        "B_wq": _B_in["wq"],
        "B_wo": _B_in["wo"],
    }

def _fwd_reference(A_x, A_k_cache, A_v_cache, A_wq, A_wo, B_x, B_k_cache, B_v_cache, B_wq, B_wo):
    def _A_ref(x, k_cache, v_cache, wq, wo):
        B, Sq, D = x.shape
        Hq, Dh = 16, 256
        Hkv, Sk = k_cache.shape[1], k_cache.shape[2]
        W = min(4096, max(256, Sk // 4))
        rep = Hq // Hkv
        q = (lambda x, *d: x.transpose(*d))((x @ wq).reshape(B, Sq, Hq, Dh), 0, 2, 1, 3)
        k = jnp.repeat(k_cache[:, :, Sk - W:, :], rep, axis=1)
        v = jnp.repeat(v_cache[:, :, Sk - W:, :], rep, axis=1)
        scores = jnp.einsum("bhqd,bhkd->bhqk", q, k) * (Dh ** -0.5)
        p = _softmax(scores, axis=-1)
        o = jnp.einsum("bhqk,bhkd->bhqd", p, v)
        return (lambda x, *d: x.transpose(*d))(o, 0, 2, 1, 3).reshape(B, Sq, Hq * Dh) @ wo

    def _B_ref(x, k_cache, v_cache, wq, wo):
        B, Sq, D = x.shape
        Hq, Dh = 16, 256
        Hkv, Sk = k_cache.shape[1], k_cache.shape[2]
        W = min(4096, max(256, Sk // 4))
        rep = Hq // Hkv
        q = (lambda x, *d: x.transpose(*d))((x @ wq).reshape(B, Sq, Hq, Dh), 0, 2, 1, 3)
        k = jnp.repeat(k_cache[:, :, Sk - W:, :], rep, axis=1)
        v = jnp.repeat(v_cache[:, :, Sk - W:, :], rep, axis=1)
        scores = jnp.einsum("bhqd,bhkd->bhqk", q, k) * (Dh ** -0.5)
        p = _softmax(scores, axis=-1)
        o = jnp.einsum("bhqk,bhkd->bhqd", p, v)
        return (lambda x, *d: x.transpose(*d))(o, 0, 2, 1, 3).reshape(B, Sq, Hq * Dh) @ wo

    a = _A_ref(A_x, A_k_cache, A_v_cache, A_wq, A_wo)
    b = _B_ref(B_x, B_k_cache, B_v_cache, B_wq, B_wo)
    return jnp.concatenate([a, b], axis=-1)


def setup_inputs():
    _inp = _fwd_setup_inputs()
    _gk = jax.random.fold_in(jax.random.key(int.from_bytes(__import__("os").urandom(4), "little")), 2**31 - 1)
    _shapes = [[2, 1, 896]]
    _dtypes = ['bfloat16']
    _gks = jax.random.split(_gk, len(_shapes))
    _gs = [jax.random.normal(k, s, dtype=jnp.dtype(d)) * 0.05 for k, s, d in zip(_gks, _shapes, _dtypes)]
    _inp["grad_out"] = _gs[0]
    return _inp

def reference(A_x, A_k_cache, A_v_cache, A_wq, A_wo, B_x, B_k_cache, B_v_cache, B_wq, B_wo, grad_out):
    _const = dict()
    def _f(*_d):
        return _fwd_reference(**{'A_x': _d[0], 'A_k_cache': _d[1], 'A_v_cache': _d[2], 'A_wq': _d[3], 'A_wo': _d[4], 'B_x': _d[5], 'B_k_cache': _d[6], 'B_v_cache': _d[7], 'B_wq': _d[8], 'B_wo': _d[9], **_const})
    _out, _vjp = jax.vjp(_f, A_x, A_k_cache, A_v_cache, A_wq, A_wo, B_x, B_k_cache, B_v_cache, B_wq, B_wo)
    _grads = _vjp(grad_out)
    _out0 = jnp.asarray(_out)
    return (_out0, *[jnp.asarray(_g) for _g in _grads])
```

```python
import functools
import jax
import jax.numpy as jnp
from jax import lax
import jax.experimental.pallas as pl
import jax.experimental.pallas.tpu as pltpu

B, D = 2, 448
HQ, HKV, SK, DH = 16, 8, 4096, 256
W = min(4096, max(256, SK // 4))
Z = SK - W
NU = B * HKV
HD = HQ * DH
SCALE = DH ** -0.5
F32, BF16 = jnp.float32, jnp.bfloat16
NT = (((1,), (1,)), ((), ()))
NN = (((1,), (0,)), ((), ()))


def make(C=32, NH=2, PC=512, units_in_p1=16, lead=1, bounds=False, rp=0, wp=0, small_first=False):
    ZSTEPS = Z // C
    WSTEPS = W // C

    def kernel(xa, ka, va, wqa, woa, xb, kb, vb, wqb, wob, g,
               out, dxa, dka, dva, dwqa, dwoa, dxb, dkb, dvb, dwqb, dwob,
               x_v, g_v, w_v, k_v, v_v, dk_v, dv_v, dw_v, zero_v,
               ls_v, ld_v, r_v, res_v, flat_v, out_v, dx_v,
               s_in, s_out):
        xs, ks, vs, wqs, wos = (xa, xb), (ka, kb), (va, vb), (wqa, wqb), (woa, wob)
        dxs, dks, dvs, dwqs, dwos = (dxa, dxb), (dka, dkb), (dva, dvb), (dwqa, dwqb), (dwoa, dwob)
        NG = NU // NH

        def small_cp(i):
            src = (xa, xb, g)[i]
            dst = (x_v.at[0], x_v.at[1], g_v)[i]
            return pltpu.make_async_copy(src, dst, s_in.at[i])

        def w_cp(br, i):
            return pltpu.make_async_copy((wqs, wos)[i][br], w_v.at[br, i], s_in.at[3 + 2 * br + i])

        def kv_cp(br, i, grp):
            b, h0 = (grp * NH) // HKV, (grp * NH) % HKV
            src = (ks, vs)[i][br].at[b, pl.ds(h0, NH), pl.ds(Z, W), :]
            dst = (k_v, v_v)[i].at[br, pl.ds(grp * NH, NH)]
            return pltpu.make_async_copy(src, dst, s_in.at[7 + (br * NG + grp) * 2 + i])

        if small_first:
            for i in range(3):
                small_cp(i).start()
        w_cp(0, 0).start(priority=rp)
        if not small_first:
            for i in range(3):
                small_cp(i).start()
        w_cp(0, 1).start(priority=rp)
        for grp in range(NG):
            kv_cp(0, 0, grp).start(priority=rp)
            kv_cp(0, 1, grp).start(priority=rp)
        w_cp(1, 0).start(priority=rp)
        w_cp(1, 1).start(priority=rp)
        for grp in range(NG):
            kv_cp(1, 0, grp).start(priority=rp)
            kv_cp(1, 1, grp).start(priority=rp)

        zero_v[...] = jnp.zeros_like(zero_v)
        ls_v[...] = jnp.zeros_like(ls_v)
        ld_v[...] = jnp.zeros_like(ld_v)
        r_v[...] = jnp.zeros_like(r_v)
        flat_v[...] = jnp.zeros_like(flat_v)

        big_out = (dka, dva, dkb, dvb)

        def zero_cp(o, i):
            b, s = i // ZSTEPS, i % ZSTEPS
            r = pl.multiple_of(s * C, C)
            return pltpu.make_async_copy(zero_v, big_out[o].at[b, :, pl.ds(r, C), :], s_out.at[o])

        def win_cp(o, i):
            b, s = i // WSTEPS, i % WSTEPS
            r = pl.multiple_of(s * C, C)
            src = (dk_v, dv_v)[o % 2].at[o // 2, pl.ds(pl.multiple_of(b * HKV, HKV), HKV), pl.ds(r, C), :]
            return pltpu.make_async_copy(src, big_out[o].at[b, :, pl.ds(Z + r, C), :], s_out.at[o])

        def dw_cp(br, j, i):
            r = pl.multiple_of((i // 4) * 8, 8)
            c = pl.multiple_of((i % 4) * 1024, 1024)
            dst = (dwqs, dwos)[j][br]
            return pltpu.make_async_copy(dw_v.at[br, j, :, pl.ds(r, 8), pl.ds(c, 1024)],
                                         dst.at[:, pl.ds(r, 8), pl.ds(c, 1024)], s_out.at[4 + 2 * br + j])

        def issue(fn, lo, n):
            def body(i, c):
                fn(lo + i).start(priority=wp)
                return c
            lax.fori_loop(0, n, body, 0)

        def rows8(v):
            v = v.astype(F32)
            return jnp.concatenate([v, jnp.zeros((6, v.shape[1]), F32)], axis=0)

        def xg(br):
            x8 = rows8(x_v[br])
            g8 = rows8(g_v[...])[:, br * D:(br + 1) * D]
            return x8, g8

        def proj(br):
            x8, g8 = xg(br)
            x8, g8 = x8.astype(BF16), g8.astype(BF16)
            for kvh in range(HKV):
                cs = pl.ds(kvh * 2 * DH, 2 * DH)
                q = lax.dot_general(x8, w_v[br, 0, :, cs], NN, preferred_element_type=F32)
                do = lax.dot_general(g8, w_v[br, 1, :, cs], NN, preferred_element_type=F32)
                q = q.astype(BF16).astype(F32)
                do = do.astype(BF16).astype(F32)
                for b in range(B):
                    u = b * HKV + kvh
                    for j in range(2):
                        qj = q[b:b + 1, j * DH:(j + 1) * DH]
                        dj = do[b:b + 1, j * DH:(j + 1) * DH]
                        ls_v[br, u, j:j + 1, :] = qj
                        ls_v[br, u, 2 + j:3 + j, :] = qj
                        ld_v[br, u, 2 + j:3 + j, :] = dj
                        r_v[br, u, j:j + 1, 0:DH] = dj
                        r_v[br, u, 2 + j:3 + j, DH:2 * DH] = qj

        def unit(br, u):
            k = k_v[br, u]
            v = v_v[br, u]
            s = lax.dot_general(ls_v[br, u].astype(BF16), k, NT, preferred_element_type=F32) * SCALE
            dp = lax.dot_general(ld_v[br, u].astype(BF16), v, NT, preferred_element_type=F32)
            m = jnp.max(s, axis=-1, keepdims=True)
            e = jnp.exp(s - m)
            p = e / jnp.sum(e, axis=-1, keepdims=True)
            ds = p * (dp - jnp.sum(p * dp, axis=-1, keepdims=True)) * SCALE
            row = lax.broadcasted_iota(jnp.int32, p.shape, 0)
            p4 = jnp.where(row < 2, p, ds)
            p4b = p4.astype(BF16)
            res_v[br, u, :, 0:DH] = lax.dot_general(p4b, v, NN, preferred_element_type=F32)
            res_v[br, u, :, DH:2 * DH] = lax.dot_general(p4b, k, NN, preferred_element_type=F32)
            p4t = p4.T.astype(BF16)
            r = r_v[br, u].astype(BF16)
            dv_v[br, u] = lax.dot_general(p4t, r[:, 0:DH], NN, preferred_element_type=F32).astype(BF16)
            dk_v[br, u] = lax.dot_general(p4t, r[:, DH:2 * DH], NN, preferred_element_type=F32).astype(BF16)

        def gather(br):
            for b in range(B):
                for kvh in range(HKV):
                    u = b * HKV + kvh
                    for j in range(2):
                        cs = pl.ds((2 * kvh + j) * DH, DH)
                        flat_v[br, 0, b:b + 1, cs] = res_v[br, u, 2 + j:3 + j, DH:2 * DH]
                        flat_v[br, 1, b:b + 1, cs] = res_v[br, u, j:j + 1, 0:DH]

        def back(br, j):
            acc = jnp.zeros((8, D), F32)
            for c in range(HD // PC):
                cs = pl.ds(c * PC, PC)
                acc += lax.dot_general(flat_v[br, j, :, cs].astype(BF16), w_v[br, j, :, cs], NT,
                                       preferred_element_type=F32)
            return acc[0:B]

        def dweight(br, j):
            a8 = xg(br)[j]
            at = a8.T.astype(BF16)
            def body(c, carry):
                cs = pl.ds(pl.multiple_of(c * PC, PC), PC)
                r = lax.dot_general(at, flat_v[br, j, :, cs].astype(BF16), NN, preferred_element_type=F32)
                dw_v[br, j, :, :, cs] = r.astype(BF16).reshape(7, 64, PC)
                return carry
            lax.fori_loop(0, HD // PC, body, 0)

        for i in range(3):
            small_cp(i).wait()
        w_cp(0, 0).wait()
        w_cp(0, 1).wait()
        proj(0)

        def grp_a(grp, c):
            kv_cp(0, 0, grp).wait()
            kv_cp(0, 1, grp).wait()
            def ub(i, c2):
                unit(0, grp * NH + i)
                return c2
            return lax.fori_loop(0, NH, ub, c)
        lax.fori_loop(0, NG, grp_a, 0)

        w_cp(1, 0).wait()
        w_cp(1, 1).wait()
        rd = [(i, grp) for grp in range(NG) for i in range(2)]
        for i, grp in rd[:len(rd) - lead]:
            kv_cp(1, i, grp).wait()
        issue(functools.partial(win_cp, 0), 0, B * WSTEPS)
        for i, grp in rd[len(rd) - lead:]:
            kv_cp(1, i, grp).wait()
        proj(1)

        per = B * ZSTEPS // NU
        def unit_b(u, c):
            issue(functools.partial(zero_cp, 0), u * per, per)
            issue(functools.partial(zero_cp, 1), u * per, per)
            unit(1, u)
            return c
        lax.fori_loop(0, NU, unit_b, 0)

        per = B * ZSTEPS // 8
        nxt = iter(range(8))
        def top_up():
            issue(functools.partial(zero_cp, 2), next(nxt) * per, per)
        outs = []
        for br in range(2):
            top_up()
            gather(br)
            dx_v[br] = back(br, 0).astype(BF16)
            top_up()
            outs.append(back(br, 1))
            top_up()
            dweight(br, 0)
            top_up()
            dweight(br, 1)
        out_v[...] = jnp.concatenate(outs, axis=1).astype(BF16)
        small_out = [pltpu.make_async_copy(out_v, out, s_out.at[8]),
                     pltpu.make_async_copy(dx_v.at[0], dxa, s_out.at[9]),
                     pltpu.make_async_copy(dx_v.at[1], dxb, s_out.at[10])]
        for cp in small_out:
            cp.start()
        for br in range(2):
            for j in range(2):
                issue(functools.partial(dw_cp, br, j), 0, 32)
        for o in range(1, 4):
            issue(functools.partial(win_cp, o), 0, B * WSTEPS)
        issue(functools.partial(zero_cp, 3), 0, B * ZSTEPS)

        for cp in small_out:
            cp.wait()
        for br in range(2):
            for j in range(2):
                dst = (dwqs, dwos)[j][br]
                pltpu.make_async_copy(dst, dst, s_out.at[4 + 2 * br + j]).wait()
        for o in range(4):
            pltpu.make_async_copy(big_out[o], big_out[o], s_out.at[o]).wait()

    any_spec = pl.BlockSpec(memory_space=pl.ANY)
    sds = jax.ShapeDtypeStruct
    br_out = [sds((B, D), BF16), sds((B, HKV, SK, DH), BF16), sds((B, HKV, SK, DH), BF16),
              sds((7, 64, HD), BF16), sds((7, 64, HD), BF16)]
    call = pl.pallas_call(
        kernel,
        out_shape=[sds((B, 2 * D), BF16)] + br_out + br_out,
        in_specs=[any_spec] * 11,
        out_specs=[any_spec] * 11,
        scratch_shapes=[
            pltpu.VMEM((2, B, D), BF16),
            pltpu.VMEM((B, 2 * D), BF16),
            pltpu.VMEM((2, 2, D, HD), BF16),
            pltpu.VMEM((2, NU, W, DH), BF16),
            pltpu.VMEM((2, NU, W, DH), BF16),
            pltpu.VMEM((2, NU, W, DH), BF16),
            pltpu.VMEM((2, NU, W, DH), BF16),
            pltpu.VMEM((2, 2, 7, 64, HD), BF16),
            pltpu.VMEM((HKV, C, DH), BF16),
            pltpu.VMEM((2, NU, 8, DH), F32),
            pltpu.VMEM((2, NU, 8, DH), F32),
            pltpu.VMEM((2, NU, 8, 2 * DH), F32),
            pltpu.VMEM((2, NU, 8, 2 * DH), F32),
            pltpu.VMEM((2, 2, 8, HD), F32),
            pltpu.VMEM((B, 2 * D), BF16),
            pltpu.VMEM((2, B, D), BF16),
            pltpu.SemaphoreType.DMA((7 + 2 * 2 * (NU // NH),)),
            pltpu.SemaphoreType.DMA((11,)),
        ],
        compiler_params=pltpu.CompilerParams(vmem_limit_bytes=110 * 1024 * 1024,
                                             disable_bounds_checks=not bounds),
    )

    @jax.jit
    def pallas_concat_heads__sliding_block_cached__sliding_block_cached__decode_kernel(A_x, A_k_cache, A_v_cache, A_wq, A_wo, B_x, B_k_cache, B_v_cache, B_wq, B_wo, grad_out):
        o = call(A_x.reshape(B, D), A_k_cache, A_v_cache, A_wq, A_wo.T,
                 B_x.reshape(B, D), B_k_cache, B_v_cache, B_wq, B_wo.T, grad_out.reshape(B, 2 * D))
        def fix(dx, dk, dv, dwq, dwo):
            return (dx.reshape(B, 1, D), dk, dv, dwq.reshape(D, HD), dwo.reshape(D, HD).T)
        return (o[0].reshape(B, 1, 2 * D), *fix(*o[1:6]), *fix(*o[6:11]))
    return pallas_concat_heads__sliding_block_cached__sliding_block_cached__decode_kernel


pallas_concat_heads__sliding_block_cached__sliding_block_cached__decode_kernel = make()
```

```python
import functools
import jax
import jax.numpy as jnp
from jax import lax
import jax.experimental.pallas as pl
import jax.experimental.pallas.tpu as pltpu

B, D = 2, 448
HQ, HKV, SK, DH = 16, 8, 4096, 256
W = min(4096, max(256, SK // 4))
Z = SK - W
NU = B * HKV
HD = HQ * DH
SCALE = DH ** -0.5
F32, BF16 = jnp.float32, jnp.bfloat16
NT = (((1,), (1,)), ((), ()))
NN = (((1,), (0,)), ((), ()))
HALF = SK // 2


def make(C=32, PC=512, INF=24, SH=4, lead=4, bounds=False, groups=(6, 6, 6, 7, 7), zgroups=(6, 6, 6, 7, 7),
         DWC=1024, scopes=False, WN=2, RC=8, first=8, q0=56, dwlast=False, do_read=True, do_write=True, do_compute=True):
    import contextlib
    scope = jax.named_scope if scopes else (lambda name: contextlib.nullcontext())
    NMAIN = W // RC
    WR = D // WN
    WCOL = (NU * RC * DH // 2) // (WN * 8)
    WPR = HD // WCOL
    NHP = (WR // 8) * WPR
    assert NHP * 8 == NMAIN * 7
    STEPS = W // C

    def kernel(xa, ka, va, wqa, woa, xb, kb, vb, wqb, wob, g,
               out, dxa, dka, dva, dwqa, dwoa, dxb, dkb, dvb, dwqb, dwob,
               x_v, g_v, w_v, kv_v, dkv_v, dw_v, zero_v,
               ls_v, ld_v, r_v, res_v, flat_v, out_v, dx_v,
               s_in, s_out):
        kv_in = (ka, va, kb, vb)
        w_in = (wqa, woa, wqb, wob)
        big_out = (dka, dva, dkb, dvb)
        dw_out = (dwqa, dwoa, dwqb, dwob)

        def small_cp(i):
            src = (xa, xb, g)[i]
            dst = (x_v.at[0], x_v.at[1], g_v)[i]
            return pltpu.make_async_copy(src, dst, s_in.at[5 + i])

        def main_cp(a, i):
            r = pl.multiple_of(i * RC, RC)
            return pltpu.make_async_copy(kv_in[a].at[:, pl.ds(Z + r, RC), :],
                                         kv_v.at[a, :, pl.ds(r, RC), :], s_in.at[0])

        def hp_cp(a, j):
            r = pl.multiple_of((j // WPR) * 8, 8)
            c = pl.multiple_of((j % WPR) * WCOL, WCOL)
            return pltpu.make_async_copy(w_in[a].at[:, pl.ds(r, 8), pl.ds(c, WCOL)],
                                         w_v.at[a, :, pl.ds(r, 8), pl.ds(c, WCOL)], s_in.at[1 + a])

        TOT = 4 * NMAIN

        def read_steps(lo, hi):
            if not do_read:
                return
            cuts = {lo, hi}
            for a in range(5):
                for c in (a * NMAIN, a * NMAIN + INF - SH, INF):
                    if lo < c < hi:
                        cuts.add(c)
            cuts = sorted(cuts)
            for s0, s1 in zip(cuts[:-1], cuts[1:]):
                def body(s, carry, s0=s0):
                    if s0 >= INF:
                        main_cp(0, 0).wait()
                    if s0 < TOT:
                        a = s0 // NMAIN
                        main_cp(a, s - a * NMAIN).start(priority=1)
                    h0 = s0 - INF + SH
                    if 0 <= h0 < TOT:
                        a = h0 // NMAIN
                        h = s - INF + SH - a * NMAIN
                        @pl.when(h % 8 != 7)
                        def _():
                            hp_cp(a, h - h // 8).start(priority=0)
                    return carry
                lax.fori_loop(s0, s1, body, 0)

        def zero_start(o, i):
            gidx, s = i // STEPS, i % STEPS
            r = pl.multiple_of(s * C, C)
            sizes = sorted(set(zgroups))
            g0 = h0 = 0
            for n in sizes:
                cnt = zgroups.count(n)
                def go(n=n, g0=g0, h0=h0):
                    pltpu.make_async_copy(
                        zero_v.at[pl.ds(0, n)],
                        big_out[o].at[pl.ds(h0 + (gidx - g0) * n, n), pl.ds(r, C), :], s_out.at[o]).start()
                if len(sizes) == 1:
                    go()
                else:
                    pl.when(jnp.logical_and(gidx >= g0, gidx < g0 + cnt))(go)
                g0 += cnt
                h0 += cnt * n
            assert h0 == 2 * NU

        def zero_issue(o, lo, n):
            if not do_write:
                return
            def body(i, c):
                zero_start(o, lo + i)
                return c
            lax.fori_loop(0, n, body, 0)

        def mixed_issue(o):
            if not do_write:
                return
            h0 = 0
            for n in groups:
                def body(s, carry, h0=h0, n=n):
                    r = pl.multiple_of(s * C, C)
                    for h in range(h0, h0 + n):
                        src = dkv_v.at[o, h // 2, pl.ds(r, C), :] if h % 2 else zero_v.at[0]
                        pltpu.make_async_copy(src, big_out[o].at[h, pl.ds(W + r, C), :], s_out.at[o]).start()
                    return carry
                lax.fori_loop(0, STEPS, body, 0)
                h0 += n
            assert h0 == 2 * NU

        def dw_issue(br):
            if not do_write:
                return
            npr = HD // DWC
            for par in range(2):
                def body(i, carry, par=par):
                    r = pl.multiple_of((i // npr) * 8, 8)
                    c = pl.multiple_of((i % npr) * DWC, DWC)
                    for a, p in ((2 * br, par), (2 * br + 1, 1 - par)):
                        for blk in range(p, 7, 2):
                            pltpu.make_async_copy(dw_v.at[a, blk, pl.ds(r, 8), pl.ds(c, DWC)],
                                                  dw_out[a].at[blk, pl.ds(r, 8), pl.ds(c, DWC)],
                                                  s_out.at[4 + a]).start()
                    return carry
                lax.fori_loop(0, 8 * npr, body, 0)

        def issue(fn, lo, n):
            def body(i, c):
                fn(lo + i).start()
                return c
            lax.fori_loop(0, n, body, 0)

        def rows8(v):
            v = v.astype(F32)
            return jnp.concatenate([v, jnp.zeros((6, v.shape[1]), F32)], axis=0)

        def xg(br):
            x8 = rows8(x_v[br])
            g8 = rows8(g_v[...])[:, br * D:(br + 1) * D]
            return x8, g8

        def wcols(a, cs):
            w = w_v[a, :, :, cs]
            return w.reshape(D, w.shape[-1])

        def proj(br):
            if not do_compute:
                return
            x8, g8 = xg(br)
            x8, g8 = x8.astype(BF16), g8.astype(BF16)
            for kvh in range(HKV):
                cs = pl.ds(kvh * 2 * DH, 2 * DH)
                q = lax.dot_general(x8, wcols(2 * br, cs), NN, preferred_element_type=F32)
                do = lax.dot_general(g8, wcols(2 * br + 1, cs), NN, preferred_element_type=F32)
                for b in range(B):
                    u = b * HKV + kvh
                    for j in range(2):
                        qj = q[b:b + 1, j * DH:(j + 1) * DH]
                        dj = do[b:b + 1, j * DH:(j + 1) * DH]
                        ls_v[br, u, j:j + 1, :] = qj
                        ls_v[br, u, 2 + j:3 + j, :] = qj
                        ld_v[br, u, 2 + j:3 + j, :] = dj
                        r_v[br, u, j:j + 1, 0:DH] = dj
                        r_v[br, u, 2 + j:3 + j, DH:2 * DH] = qj

        def unit(br, u):
            if not do_compute:
                return
            k = kv_v[2 * br, u]
            v = kv_v[2 * br + 1, u]
            s = lax.dot_general(ls_v[br, u].astype(BF16), k, NT, preferred_element_type=F32) * SCALE
            dp = lax.dot_general(ld_v[br, u].astype(BF16), v, NT, preferred_element_type=F32)
            m = jnp.max(s, axis=-1, keepdims=True)
            e = jnp.exp(s - m)
            p = e / jnp.sum(e, axis=-1, keepdims=True)
            ds = p * (dp - jnp.sum(p * dp, axis=-1, keepdims=True)) * SCALE
            row = lax.broadcasted_iota(jnp.int32, p.shape, 0)
            p4 = jnp.where(row < 2, p, ds)
            p4b = p4.astype(BF16)
            res_v[br, u, :, 0:DH] = lax.dot_general(p4b, v, NN, preferred_element_type=F32)
            res_v[br, u, :, DH:2 * DH] = lax.dot_general(p4b, k, NN, preferred_element_type=F32)
            p4t = p4.T.astype(BF16)
            r = r_v[br, u].astype(BF16)
            dkv_v[2 * br + 1, u] = lax.dot_general(p4t, r[:, 0:DH], NN, preferred_element_type=F32).astype(BF16)
            dkv_v[2 * br, u] = lax.dot_general(p4t, r[:, DH:2 * DH], NN, preferred_element_type=F32).astype(BF16)

        def gather(br):
            if not do_compute:
                return
            for b in range(B):
                for kvh in range(HKV):
                    u = b * HKV + kvh
                    for j in range(2):
                        cs = pl.ds((2 * kvh + j) * DH, DH)
                        flat_v[br, 0, b:b + 1, cs] = res_v[br, u, 2 + j:3 + j, DH:2 * DH]
                        flat_v[br, 1, b:b + 1, cs] = res_v[br, u, j:j + 1, 0:DH]

        def back(br, j):
            acc = jnp.zeros((8, D), F32)
            for c in range(HD // PC if do_compute else 0):
                cs = pl.ds(c * PC, PC)
                acc += lax.dot_general(flat_v[br, j, :, cs].astype(BF16), wcols(2 * br + j, cs), NT,
                                       preferred_element_type=F32)
            return acc[0:B]

        def dweight(br, j):
            if not do_compute:
                return
            a8 = xg(br)[j]
            at = a8.T.astype(BF16)
            def body(c, carry):
                cs = pl.ds(pl.multiple_of(c * PC, PC), PC)
                r = lax.dot_general(at, flat_v[br, j, :, cs].astype(BF16), NN, preferred_element_type=F32)
                dw_v[2 * br + j, :, :, cs] = r.astype(BF16).reshape(7, 64, PC)
                return carry
            lax.fori_loop(0, HD // PC, body, 0)

        with scope("reads0"):
            read_steps(0, INF)
        for i in range(3):
            small_cp(i).start()
        zero_v[...] = jnp.zeros_like(zero_v)
        with scope("reads"):
            read_steps(INF, TOT + INF - lead)
        NZ = len(zgroups) * STEPS
        with scope("issue0"):
            zero_issue(0, 0, first)
            read_steps(TOT + INF - lead, TOT + INF)
            zero_issue(0, first, q0 - first)
        with scope("wait_rest"):
            for a in range(4 if do_read else 0):
                pltpu.make_async_copy(w_in[a], w_v.at[a], s_in.at[1 + a]).wait()
            for i in range(3):
                small_cp(i).wait()

        ls_v[...] = jnp.zeros_like(ls_v)
        ld_v[...] = jnp.zeros_like(ld_v)
        r_v[...] = jnp.zeros_like(r_v)
        flat_v[...] = jnp.zeros_like(flat_v)

        per = NZ // NU
        def units(br):
            def body(u, c):
                with scope("issue_u"):
                    zero_issue(1 + br, u * per, per)
                with scope("unit"):
                    unit(br, u)
                return c
            lax.fori_loop(0, NU, body, 0)

        rest = NZ - q0
        t0, t1 = rest // 4, (rest * 5) // 8
        proj(0)
        zero_issue(0, q0, t0)
        units(0)
        zero_issue(0, q0 + t0, t1 - t0)
        proj(1)
        zero_issue(0, q0 + t1, rest - t1)
        units(1)

        nxt = iter(range(8))
        def top_up():
            with scope("topup"):
                zero_issue(3, next(nxt) * (NZ // 8), NZ // 8)
        outs = []
        for br in range(2):
            top_up()
            gather(br)
            dx_v[br] = back(br, 0).astype(BF16)
            top_up()
            outs.append(back(br, 1))
            top_up()
            dweight(br, 0)
            top_up()
            dweight(br, 1)
        out_v[...] = jnp.concatenate(outs, axis=1).astype(BF16)
        small_out = [pltpu.make_async_copy(out_v, out, s_out.at[8]),
                     pltpu.make_async_copy(dx_v.at[0], dxa, s_out.at[9]),
                     pltpu.make_async_copy(dx_v.at[1], dxb, s_out.at[10])]
        for cp in small_out:
            cp.start()
        if not dwlast:
            with scope("issue_dw"):
                for br in range(2):
                    dw_issue(br)
        with scope("issue_mixed"):
            for o in range(4):
                mixed_issue(o)
        if dwlast:
            with scope("issue_dw"):
                for br in range(2):
                    dw_issue(br)

        with scope("final"):
            for cp in small_out:
                cp.wait()
            for a in range(4 if do_write else 0):
                pltpu.make_async_copy(dw_out[a], dw_out[a], s_out.at[4 + a]).wait()
            for o in range(4 if do_write else 0):
                pltpu.make_async_copy(big_out[o], big_out[o], s_out.at[o]).wait()

    any_spec = pl.BlockSpec(memory_space=pl.ANY)
    sds = jax.ShapeDtypeStruct
    br_out = [sds((B, D), BF16), sds((2 * NU, HALF, DH), BF16), sds((2 * NU, HALF, DH), BF16),
              sds((7, 64, HD), BF16), sds((7, 64, HD), BF16)]
    call = pl.pallas_call(
        kernel,
        out_shape=[sds((B, 2 * D), BF16)] + br_out + br_out,
        in_specs=[any_spec] * 11,
        out_specs=[any_spec] * 11,
        scratch_shapes=[
            pltpu.VMEM((2, B, D), BF16),
            pltpu.VMEM((B, 2 * D), BF16),
            pltpu.VMEM((4, WN, WR, HD), BF16),
            pltpu.VMEM((4, NU, W, DH), BF16),
            pltpu.VMEM((4, NU, W, DH), BF16),
            pltpu.VMEM((4, 7, 64, HD), BF16),
            pltpu.VMEM((8, C, DH), BF16),
            pltpu.VMEM((2, NU, 8, DH), F32),
            pltpu.VMEM((2, NU, 8, DH), F32),
            pltpu.VMEM((2, NU, 8, 2 * DH), F32),
            pltpu.VMEM((2, NU, 8, 2 * DH), F32),
            pltpu.VMEM((2, 2, 8, HD), F32),
            pltpu.VMEM((B, 2 * D), BF16),
            pltpu.VMEM((2, B, D), BF16),
            pltpu.SemaphoreType.DMA((8,)),
            pltpu.SemaphoreType.DMA((11,)),
        ],
        compiler_params=pltpu.CompilerParams(vmem_limit_bytes=110 * 1024 * 1024,
                                             disable_bounds_checks=not bounds),
    )

    @jax.jit
    def pallas_concat_heads__sliding_block_cached__sliding_block_cached__decode_kernel(A_x, A_k_cache, A_v_cache, A_wq, A_wo, B_x, B_k_cache, B_v_cache, B_wq, B_wo, grad_out):
        def prep(x, k, v, wq, wo):
            return (x.reshape(B, D), k.reshape(NU, SK, DH), v.reshape(NU, SK, DH),
                    wq.reshape(WN, WR, HD), wo.T.reshape(WN, WR, HD))
        o = call(*prep(A_x, A_k_cache, A_v_cache, A_wq, A_wo), *prep(B_x, B_k_cache, B_v_cache, B_wq, B_wo),
                 grad_out.reshape(B, 2 * D))
        def fix(dx, dk, dv, dwq, dwo):
            return (dx.reshape(B, 1, D), dk.reshape(B, HKV, SK, DH), dv.reshape(B, HKV, SK, DH),
                    dwq.reshape(D, HD), dwo.reshape(D, HD).T)
        return (o[0].reshape(B, 1, 2 * D), *fix(*o[1:6]), *fix(*o[6:11]))
    return pallas_concat_heads__sliding_block_cached__sliding_block_cached__decode_kernel


pallas_concat_heads__sliding_block_cached__sliding_block_cached__decode_kernel = make()
```

```python
import jax
import jax.numpy as jnp
from jax import lax
import jax.experimental.pallas as pl
import jax.experimental.pallas.tpu as pltpu

B, D = 2, 448
HQ, HKV, SK, DH = 16, 8, 4096, 256
W = min(4096, max(256, SK // 4))
Z = SK - W
NU = B * HKV
HD = HQ * DH
HALF = SK // 2
SCALE = DH ** -0.5
F32, BF16 = jnp.float32, jnp.bfloat16
NT = (((1,), (1,)), ((), ()))
NN = (((1,), (0,)), ((), ()))
assert HQ == 2 * HKV and HALF == 2 * W

INFLIGHT = 14
AHEAD = 2
LEAD = 3
RC = 8
NMAIN = W // RC
TOT = 4 * NMAIN
WN, WR, WCOL = 2, D // 2, 1024
WPR = HD // WCOL
assert (WR // 8) * WPR * 8 == NMAIN * 7
GROUPS = (6, 6, 6, 7, 7)
FIRST, Q0, Q1, Q2 = 8, 60, 92, 126
C = 32
STEPS = W // C
NZ = len(GROUPS) * STEPS
NB, BR, DWC = 7, 64, 1024
PC = 512
assert sum(GROUPS) == 2 * NU and tuple(sorted(GROUPS)) == GROUPS
KV_SEMS = 16
S_W, S_SMALL_IN, N_IN = KV_SEMS, KV_SEMS + 4, KV_SEMS + 7
S_ZERO, S_DW, S_SMALL_OUT, S_RUN, N_OUT = 0, 4, 8, 11, 13
assert INFLIGHT <= KV_SEMS and NMAIN % KV_SEMS == 0


def kernel(xa, ka, va, wqa, woa, xb, kb, vb, wqb, wob, g,
           out, dxa, dka, dva, dwqa, dwoa, dxb, dkb, dvb, dwqb, dwob,
           x_v, g_v, w_v, kv_v, dkv_v, dw_v, zero_v,
           ls_v, ld_v, r_v, res_v, flat_v, out_v, dx_v,
           s_in, s_out):
    kv_in = (ka, va, kb, vb)
    w_in = (wqa, woa, wqb, wob)
    dkv_out = (dka, dva, dkb, dvb)
    dw_out = (dwqa, dwoa, dwqb, dwob)
    copy = pltpu.make_async_copy

    def wait_filled(ref, sem):
        copy(ref, ref, sem).wait()

    small_in = [copy(src, dst, s_in.at[S_SMALL_IN + i])
                for i, (src, dst) in enumerate(((xa, x_v.at[0]), (xb, x_v.at[1]), (g, g_v)))]

    def kv_read(a, i):
        r = pl.multiple_of(i * RC, RC)
        return copy(kv_in[a].at[:, pl.ds(Z + r, RC), :], kv_v.at[a, :, pl.ds(r, RC), :],
                    s_in.at[i % KV_SEMS])

    def w_read(a, j):
        r = pl.multiple_of((j // WPR) * 8, 8)
        c = pl.multiple_of((j % WPR) * WCOL, WCOL)
        return copy(w_in[a].at[:, pl.ds(r, 8), pl.ds(c, WCOL)],
                    w_v.at[a, :, pl.ds(r, 8), pl.ds(c, WCOL)], s_in.at[S_W + a])

    def read_steps(lo, hi):
        cuts = {lo, hi}
        for a in range(5):
            cuts |= {c for c in (a * NMAIN, a * NMAIN + INFLIGHT, a * NMAIN + INFLIGHT - AHEAD)
                     if lo < c < hi}
        cuts = sorted(cuts)
        for s0, s1 in zip(cuts[:-1], cuts[1:]):
            def body(s, carry, s0=s0):
                if s0 >= INFLIGHT:
                    a = (s0 - INFLIGHT) // NMAIN
                    kv_read(a, s - INFLIGHT - a * NMAIN).wait()
                if s0 < TOT:
                    a = s0 // NMAIN
                    kv_read(a, s - a * NMAIN).start(priority=1)
                if 0 <= s0 - INFLIGHT + AHEAD < TOT:
                    a = (s0 - INFLIGHT + AHEAD) // NMAIN
                    h = s - INFLIGHT + AHEAD - a * NMAIN

                    @pl.when(h % 8 != 7)
                    def _():
                        w_read(a, h - h // 8).start(priority=0)
                return carry
            lax.fori_loop(s0, s1, body, 0)

    def zero_writes(o, lo, count):
        def body(i, carry):
            grp = (lo + i) // STEPS
            r = pl.multiple_of(((lo + i) % STEPS) * C, C)
            g0 = h0 = 0
            for n in sorted(set(GROUPS)):
                cnt = GROUPS.count(n)

                @pl.when(jnp.logical_and(grp >= g0, grp < g0 + cnt))
                def _(n=n, g0=g0, h0=h0):
                    copy(zero_v.at[pl.ds(0, n)],
                         dkv_out[o].at[pl.ds(h0 + (grp - g0) * n, n), pl.ds(r, C), :],
                         s_out.at[S_ZERO + o]).start()
                g0, h0 = g0 + cnt, h0 + cnt * n
            return carry
        lax.fori_loop(0, count, body, 0)

    def window_run(o, h0, n, sem):
        def body(s, carry):
            r = pl.multiple_of(s * C, C)
            for h in range(h0, h0 + n):
                src = dkv_v.at[o, h // 2, pl.ds(r, C), :] if h % 2 else zero_v.at[0]
                copy(src, dkv_out[o].at[h, pl.ds(W + r, C), :], sem).start()
            return carry
        lax.fori_loop(0, STEPS, body, 0)
        return dkv_out[o].at[pl.ds(h0, n), pl.ds(W, W), :]

    def dw_run(br, par):
        blocks = [(a, blk) for a, p in ((2 * br, par), (2 * br + 1, 1 - par)) for blk in range(p, NB, 2)]
        npr = HD // DWC

        def body(i, carry):
            r = pl.multiple_of((i // npr) * 8, 8)
            c = pl.multiple_of((i % npr) * DWC, DWC)
            for a, blk in blocks:
                copy(dw_v.at[a, blk, pl.ds(r, 8), pl.ds(c, DWC)],
                     dw_out[a].at[blk, pl.ds(r, 8), pl.ds(c, DWC)], s_out.at[S_DW + a]).start()
            return carry
        lax.fori_loop(0, (BR // 8) * npr, body, 0)

    def rows8(v):
        return jnp.concatenate([v.astype(F32), jnp.zeros((8 - B, v.shape[1]), F32)], axis=0)

    def x_and_g(br):
        return rows8(x_v[br]), rows8(g_v[...])[:, br * D:(br + 1) * D]

    def w_cols(a, cs):
        w = w_v[a, :, :, cs]
        return w.reshape(D, w.shape[-1])

    def dot(a, b, dims):
        return lax.dot_general(a, b, dims, preferred_element_type=F32)

    def project(br):
        x8, g8 = (t.astype(BF16) for t in x_and_g(br))
        for kvh in range(HKV):
            cs = pl.ds(kvh * 2 * DH, 2 * DH)
            q = dot(x8, w_cols(2 * br, cs), NN)
            do = dot(g8, w_cols(2 * br + 1, cs), NN)
            for b in range(B):
                u = b * HKV + kvh
                for j in range(2):
                    qj = q[b:b + 1, j * DH:(j + 1) * DH]
                    dj = do[b:b + 1, j * DH:(j + 1) * DH]
                    ls_v[br, u, j:j + 1, :] = qj
                    ls_v[br, u, 2 + j:3 + j, :] = qj
                    ld_v[br, u, 2 + j:3 + j, :] = dj
                    r_v[br, u, j:j + 1, 0:DH] = dj
                    r_v[br, u, 2 + j:3 + j, DH:2 * DH] = qj

    def attend(br, u):
        k = kv_v[2 * br, u]
        v = kv_v[2 * br + 1, u]
        s = dot(ls_v[br, u].astype(BF16), k, NT) * SCALE
        dp = dot(ld_v[br, u].astype(BF16), v, NT)
        e = jnp.exp(s - jnp.max(s, axis=-1, keepdims=True))
        p = e / jnp.sum(e, axis=-1, keepdims=True)
        ds = p * (dp - jnp.sum(p * dp, axis=-1, keepdims=True)) * SCALE
        row = lax.broadcasted_iota(jnp.int32, p.shape, 0)
        pd = jnp.where(row < 2, p, ds)
        pdb = pd.astype(BF16)
        res_v[br, u, :, 0:DH] = dot(pdb, v, NN)
        res_v[br, u, :, DH:2 * DH] = dot(pdb, k, NN)
        pdt = pd.T.astype(BF16)
        r = r_v[br, u].astype(BF16)
        dkv_v[2 * br + 1, u] = dot(pdt, r[:, 0:DH], NN).astype(BF16)
        dkv_v[2 * br, u] = dot(pdt, r[:, DH:2 * DH], NN).astype(BF16)

    def flatten(br):
        for b in range(B):
            for kvh in range(HKV):
                u = b * HKV + kvh
                for j in range(2):
                    cs = pl.ds((2 * kvh + j) * DH, DH)
                    flat_v[2 * br, b:b + 1, cs] = res_v[br, u, 2 + j:3 + j, DH:2 * DH]
                    flat_v[2 * br + 1, b:b + 1, cs] = res_v[br, u, j:j + 1, 0:DH]

    def contract(a):
        def body(c, acc):
            cs = pl.ds(pl.multiple_of(c * 2 * PC, 2 * PC), 2 * PC)
            return acc + dot(flat_v[a, :, cs].astype(BF16), w_cols(a, cs), NT)
        return lax.fori_loop(0, HD // (2 * PC), body, jnp.zeros((8, D), F32))[0:B]

    def weight_grad(a):
        lhs = x_and_g(a // 2)[a % 2].T.astype(BF16)

        def body(c, carry):
            cs = pl.ds(pl.multiple_of(c * PC, PC), PC)
            dw = dot(lhs, flat_v[a, :, cs].astype(BF16), NN)
            dw_v[a, :, :, cs] = dw.astype(BF16).reshape(NB, BR, PC)
            return carry
        lax.fori_loop(0, HD // PC, body, 0)

    read_steps(0, INFLIGHT)
    for cp in small_in:
        cp.start()
    zero_v[...] = jnp.zeros_like(zero_v)
    read_steps(INFLIGHT, TOT + INFLIGHT - LEAD)
    zero_writes(0, 0, FIRST)
    read_steps(TOT + INFLIGHT - LEAD, TOT + INFLIGHT)
    zero_writes(0, FIRST, Q0 - FIRST)
    for a in range(4):
        wait_filled(w_v.at[a], s_in.at[S_W + a])
    for cp in small_in:
        cp.wait()

    for ref in (ls_v, ld_v, r_v, flat_v):
        ref[...] = jnp.zeros_like(ref)

    def attend_all(br):
        def body(u, carry):
            zero_writes(1 + br, u * (NZ // NU), NZ // NU)
            attend(br, u)
            return carry
        lax.fori_loop(0, NU, body, 0)

    project(0)
    zero_writes(0, Q0, Q1 - Q0)
    attend_all(0)
    zero_writes(0, Q1, Q2 - Q1)
    project(1)
    zero_writes(0, Q2, NZ - Q2)
    attend_all(1)

    outs = []
    e = NZ // 8
    for br in range(2):
        zero_writes(3, (4 * br) * e, e)
        flatten(br)
        dx_v[br] = contract(2 * br).astype(BF16)
        zero_writes(3, (4 * br + 1) * e, e)
        outs.append(contract(2 * br + 1))
        zero_writes(3, (4 * br + 2) * e, e)
        weight_grad(2 * br)
        zero_writes(3, (4 * br + 3) * e, e)
        weight_grad(2 * br + 1)
    out_v[...] = jnp.concatenate(outs, axis=1).astype(BF16)
    small_out = [copy(src, dst, s_out.at[S_SMALL_OUT + i])
                 for i, (src, dst) in enumerate(((out_v, out), (dx_v.at[0], dxa), (dx_v.at[1], dxb)))]
    for cp in small_out:
        cp.start()

    dw_run(0, 0)
    for o in range(4):
        wait_filled(dkv_out[o].at[:, pl.ds(0, W), :], s_out.at[S_ZERO + o])
    for cp in small_out:
        cp.wait()
    dw_run(0, 1)
    dw_run(1, 0)
    dw_run(1, 1)
    pending = [(dw_out[a], s_out.at[S_DW + a]) for a in range(4)]
    runs = [(o, sum(GROUPS[:i]), n) for o in range(4) for i, n in enumerate(GROUPS)]
    for i, run in enumerate(runs):
        sem = s_out.at[S_RUN + i % 2]
        started = (window_run(*run, sem), sem)
        for ref, prev_sem in pending:
            wait_filled(ref, prev_sem)
        pending = [started]
    wait_filled(*pending[0])


@jax.jit
def pallas_concat_heads__sliding_block_cached__sliding_block_cached__decode_kernel(
        A_x, A_k_cache, A_v_cache, A_wq, A_wo, B_x, B_k_cache, B_v_cache, B_wq, B_wo, grad_out):
    def prep(x, k, v, wq, wo):
        return (x.reshape(B, D), k.reshape(NU, SK, DH), v.reshape(NU, SK, DH),
                wq.reshape(WN, WR, HD), wo.T.reshape(WN, WR, HD))

    def fix(dx, dk, dv, dwq, dwo):
        return (dx.reshape(B, 1, D), dk.reshape(B, HKV, SK, DH), dv.reshape(B, HKV, SK, DH),
                dwq.reshape(D, HD), dwo.reshape(D, HD).T)

    no_checks = {name: True for name in ("disable_bounds_checks", "disable_semaphore_checks")
                 if hasattr(pltpu.CompilerParams, name)}
    hbm = pl.BlockSpec(memory_space=pl.ANY)
    sds = jax.ShapeDtypeStruct
    grads = [sds((B, D), BF16), sds((2 * NU, HALF, DH), BF16), sds((2 * NU, HALF, DH), BF16),
             sds((NB, BR, HD), BF16), sds((NB, BR, HD), BF16)]
    o = pl.pallas_call(
        kernel,
        out_shape=[sds((B, 2 * D), BF16)] + grads + grads,
        in_specs=[hbm] * 11,
        out_specs=[hbm] * 11,
        scratch_shapes=[
            pltpu.VMEM((2, B, D), BF16),
            pltpu.VMEM((B, 2 * D), BF16),
            pltpu.VMEM((4, WN, WR, HD), BF16),
            pltpu.VMEM((4, NU, W, DH), BF16),
            pltpu.VMEM((4, NU, W, DH), BF16),
            pltpu.VMEM((4, NB, BR, HD), BF16),
            pltpu.VMEM((max(GROUPS), C, DH), BF16),
            pltpu.VMEM((2, NU, 8, DH), F32),
            pltpu.VMEM((2, NU, 8, DH), F32),
            pltpu.VMEM((2, NU, 8, 2 * DH), F32),
            pltpu.VMEM((2, NU, 8, 2 * DH), F32),
            pltpu.VMEM((4, 8, HD), F32),
            pltpu.VMEM((B, 2 * D), BF16),
            pltpu.VMEM((2, B, D), BF16),
            pltpu.SemaphoreType.DMA((N_IN,)),
            pltpu.SemaphoreType.DMA((N_OUT,)),
        ],
        compiler_params=pltpu.CompilerParams(vmem_limit_bytes=110 * 1024 * 1024, **no_checks),
    )(*prep(A_x, A_k_cache, A_v_cache, A_wq, A_wo), *prep(B_x, B_k_cache, B_v_cache, B_wq, B_wo),
      grad_out.reshape(B, 2 * D))
    return (o[0].reshape(B, 1, 2 * D), *fix(*o[1:6]), *fix(*o[6:11]))
```
